```python
import jax
import jax.numpy as jnp

def _softmax(x, axis=-1):
    return jax.nn.softmax(x, axis=axis)
def _gelu(x):
    return jax.nn.gelu(x, approximate=True)
def _silu(x):
    return jax.nn.silu(x)
def _sigmoid(x):
    return jax.nn.sigmoid(x)
def _layernorm(x, axis=-1, eps=1e-5):
    m = jnp.mean(x, axis=axis, keepdims=True)
    v = jnp.var(x, axis=axis, keepdims=True)
    return (x - m) / jnp.sqrt(v + eps)
def _scatter_add(tgt, idx, src, axis=0):
    return tgt.at[idx].add(src)
def _segment_sum(src, seg, n):
    return jax.ops.segment_sum(src, seg, n)
class _Rng:
    def __init__(self, key):
        self._k = key
    def _next(self):
        self._k, sub = jax.random.split(self._k)
        return sub
    def normal(self, shape):
        return jax.random.normal(self._next(), shape, dtype=jnp.bfloat16)
    def randint(self, lo, hi, shape):
        return jax.random.randint(self._next(), shape, lo, hi, dtype=jnp.int32)
    def uniform(self, shape, lo=0.0, hi=1.0):
        return jax.random.uniform(self._next(), shape, jnp.bfloat16, lo, hi)
    def permutation(self, n):
        return jax.random.permutation(self._next(), n)


kernel_name = 'standalone__cross_network_dcn_v2__recsys'

def setup_inputs():
    _rng = _Rng(jax.random.key(int.from_bytes(__import__("os").urandom(4), "little")))
    _w = (lambda a: (lambda t: t.astype(jnp.bfloat16) if jnp.issubdtype(t.dtype, jnp.floating) else t)(jnp.asarray(a)))
    B, F, D, L = 16384, 100, 16, 3
    Din = min(F * D, 512)
    R = max(Din // 4, 2)
    sc = Din ** -0.5
    return {
        "x0": _w((lambda *s: _rng.normal(s) * 0.05)(B, Din)),
        "U":  _w((lambda *s: _rng.normal(s) * 0.05)(L, Din, R) * sc),
        "V":  _w((lambda *s: _rng.normal(s) * 0.05)(L, R, Din) * sc),
        "bs": _w((lambda *s: _rng.normal(s) * 0.05)(L, Din)),
    }

def reference(x0, U, V, bs):
    x = x0
    for l in range(U.shape[0]):
        h = jnp.einsum('rd,bd->br', V[l], x)
        h = jnp.einsum('dr,br->bd', U[l], h)
        x = x0 * (h + bs[l]) + x
    return x
```

```python
import jax
import jax.numpy as jnp
import jax.experimental.pallas as pl
import jax.experimental.pallas.tpu as pltpu

_TB = 1024


def _cross_kernel(x0_ref, u_ref, v_ref, b_ref, o_ref):
    num_layers = u_ref.shape[0]
    x0 = x0_ref[...]
    x0f = x0.astype(jnp.float32)
    x = x0
    for l in range(num_layers):
        h = jax.lax.dot_general(
            x, v_ref[l], (((1,), (1,)), ((), ())),
            preferred_element_type=jnp.float32)
        g = jax.lax.dot_general(
            h.astype(jnp.bfloat16), u_ref[l], (((1,), (1,)), ((), ())),
            preferred_element_type=jnp.float32)
        b = b_ref[pl.ds(l, 1), :].astype(jnp.float32)
        x = (x0f * (g + b) + x.astype(jnp.float32)).astype(jnp.bfloat16)
    o_ref[...] = x


@jax.jit
def pallas_standalone__cross_network_dcn_v2__recsys_kernel(x0, U, V, bs):
    B, D = x0.shape
    L, _, R = U.shape
    tb = min(_TB, B)
    return pl.pallas_call(
        _cross_kernel,
        grid=(pl.cdiv(B, tb),),
        in_specs=[
            pl.BlockSpec((tb, D), lambda i: (i, 0)),
            pl.BlockSpec((L, D, R), lambda i: (0, 0, 0)),
            pl.BlockSpec((L, R, D), lambda i: (0, 0, 0)),
            pl.BlockSpec((L, D), lambda i: (0, 0)),
        ],
        out_specs=pl.BlockSpec((tb, D), lambda i: (i, 0)),
        out_shape=jax.ShapeDtypeStruct((B, D), x0.dtype),
        compiler_params=pltpu.CompilerParams(
            dimension_semantics=("arbitrary",),
            vmem_limit_bytes=64 * 1024 * 1024,
        ),
    )(x0, U, V, bs)
```

```python
import jax
import jax.numpy as jnp
import jax.experimental.pallas as pl
import jax.experimental.pallas.tpu as pltpu

SIZES = [320] + [256] * 14 + [192]
AHEAD = 2
NSEM = 4
FLAGS = {"XLA_TPU_RESCHEDULE_DMA_DONES": True}
NOSEMCHK = True
NOBND = True
LASTP = 3


def _kernel(x_hbm, u_hbm, v_hbm, b_hbm, o_hbm, xbuf, obuf, ubuf, vbuf, bbuf, isem, osem):
    L = u_hbm.shape[0]
    B = x_hbm.shape[0]
    nin = len(SIZES)
    tot = sum(SIZES)
    offs = [sum(SIZES[:j]) for j in range(nin)]
    nout = B // tot
    assert nin % NSEM == 0 and AHEAD < NSEM

    def row(it, off):
        if isinstance(it, int):
            return it * tot + off
        return pl.multiple_of(it * tot + off, 16)

    def xcp(it, j):
        it, j = it + j // nin, j % nin
        s = row(it, offs[j])
        return pltpu.make_async_copy(x_hbm.at[pl.ds(s, SIZES[j])], xbuf.at[pl.ds(s, SIZES[j])], isem.at[j % NSEM])

    def ocp(it, off, n):
        s = row(it, off)
        return pltpu.make_async_copy(obuf.at[pl.ds(s, n)], o_hbm.at[pl.ds(s, n)], osem.at[0])

    def wcp(k):
        l = k // 2
        if k % 2 == 0:
            return pltpu.make_async_copy(v_hbm.at[l], vbuf.at[l], isem.at[NSEM + k])
        return pltpu.make_async_copy(u_hbm.at[l], ubuf.at[l], isem.at[NSEM + k])

    bcp = pltpu.make_async_copy(b_hbm, bbuf, isem.at[NSEM + 2 * L])

    wcp(0).start()
    xcp(0, 0).start()
    wcp(1).start()
    bcp.start()
    for k in range(2, 2 * L):
        wcp(k).start()
    for c in range(1, AHEAD):
        xcp(0, c).start()

    def body(it, carry):
        first = it == 0
        for j in range(nin):
            n = SIZES[j]
            if j == 0:
                pl.when(first)(lambda: wcp(0).wait())
            xcp(it, j).wait()
            if j + AHEAD < nin:
                xcp(it, j + AHEAD).start()
            else:
                pl.when(it < nout - 1)(lambda: xcp(it, j + AHEAD).start())
            s = row(it, offs[j])
            x0 = xbuf[pl.ds(s, n), :]
            x0f = x0.astype(jnp.float32)
            x = x0
            for l in range(L):
                if j == 0 and l > 0:
                    pl.when(first)(lambda: wcp(2 * l).wait())
                h = jax.lax.dot_general(x, vbuf[l], (((1,), (1,)), ((), ())),
                                        preferred_element_type=jnp.float32)
                if j == 0:
                    pl.when(first)(lambda: wcp(2 * l + 1).wait())
                    if l == 0:
                        pl.when(first)(lambda: bcp.wait())
                g = jax.lax.dot_general(h.astype(jnp.bfloat16), ubuf[l], (((1,), (1,)), ((), ())),
                                        preferred_element_type=jnp.float32)
                b = bbuf[pl.ds(l, 1), :].astype(jnp.float32)
                x = (x0f * (g + b) + x.astype(jnp.float32)).astype(jnp.bfloat16)
            np_ = LASTP if j == nin - 1 else 1
            pn = n // np_
            for p in range(np_):
                obuf[pl.ds(row(it, offs[j] + p * pn), pn), :] = x[p * pn:(p + 1) * pn]
                ocp(it, offs[j] + p * pn, pn).start()
        return carry

    jax.lax.fori_loop(0, nout, body, 0)
    pltpu.make_async_copy(obuf, o_hbm, osem.at[0]).wait()


@jax.jit
def pallas_standalone__cross_network_dcn_v2__recsys_kernel(x0, U, V, bs):
    B, D = x0.shape
    L, _, R = U.shape
    any_spec = pl.BlockSpec(memory_space=pl.ANY)
    return pl.pallas_call(
        _kernel,
        in_specs=[any_spec] * 4,
        out_specs=any_spec,
        out_shape=jax.ShapeDtypeStruct((B, D), x0.dtype),
        scratch_shapes=[
            pltpu.VMEM((B, D), x0.dtype),
            pltpu.VMEM((B, D), x0.dtype),
            pltpu.VMEM((L, D, R), U.dtype),
            pltpu.VMEM((L, R, D), V.dtype),
            pltpu.VMEM((L, D), bs.dtype),
            pltpu.SemaphoreType.DMA((NSEM + 2 * L + 1,)),
            pltpu.SemaphoreType.DMA((1,)),
        ],
        compiler_params=pltpu.CompilerParams(vmem_limit_bytes=100 * 1024 * 1024, flags=FLAGS,
                                             disable_semaphore_checks=NOSEMCHK,
                                             disable_bounds_checks=NOBND),
    )(x0, U, V, bs)
```

```python
import jax
import jax.numpy as jnp
import jax.experimental.pallas as pl
import jax.experimental.pallas.tpu as pltpu

_SIZES = (272, 176) + (256,) * 27 + (336, 336, 160)
_IN_SEGS = (1, 1, 2) + (4,) * 7
_OUT_SEGS = (4,) * 7 + (2, 1, 1)
_LAST_PIECES = (32,) * 5
_AHEAD = 2
_SPLIT = 192
_HOLD = 32
_HOLD_NEXT = 16


def _mm(a, w):
    return jax.lax.dot_general(
        a, w, (((1,), (1,)), ((), ())), preferred_element_type=jnp.float32
    )


def _cross_kernel(
    x_hbm, u_hbm, v_hbm, b_hbm, o_hbm, xbuf, obuf, ubuf, vbuf, bbuf, isem, osem
):
    num_layers, _, rank = u_hbm.shape
    num_chunks = len(_SIZES)
    num_segs = len(_IN_SEGS)
    block = sum(_SIZES)
    num_iters = x_hbm.shape[0] // block
    offs = [sum(_SIZES[:j]) for j in range(num_chunks + 1)]
    seg_start = [sum(_IN_SEGS[:q]) for q in range(num_segs + 1)]
    out_first = {
        sum(_OUT_SEGS[: q + 1]) - 1: sum(_OUT_SEGS[:q]) for q in range(len(_OUT_SEGS))
    }

    def row(it, off):
        if isinstance(it, int):
            return it * block + off
        return pl.multiple_of(it * block + off, 16)

    def x_copy(it, q):
        it, q = it + q // num_segs, q % num_segs
        off = offs[seg_start[q]]
        rows = pl.ds(row(it, off), offs[seg_start[q + 1]] - off)
        return pltpu.make_async_copy(x_hbm.at[rows], xbuf.at[rows], isem.at[q])

    def o_copy(it, off, n):
        rows = pl.ds(row(it, off), n)
        return pltpu.make_async_copy(obuf.at[rows], o_hbm.at[rows], osem.at[0])

    def w_copy(k):
        src, dst = (v_hbm, vbuf) if k % 2 == 0 else (u_hbm, ubuf)
        return pltpu.make_async_copy(
            src.at[k // 2], dst.at[k // 2], isem.at[num_segs + k]
        )

    b_copy = pltpu.make_async_copy(b_hbm, bbuf, isem.at[num_segs + 2 * num_layers])

    def hold(val, start, n):
        spare = vbuf.at[num_layers, pl.ds(0, n), pl.ds(0, rank)]
        spare[...] = val[start : start + n, :rank]
        mid = spare[...]
        if val.shape[1] > rank:
            mid = jnp.concatenate([mid, val[start : start + n, rank:]], axis=1)
        head = [val[:start]] if start else []
        return jnp.concatenate(head + [mid, val[start + n :]], axis=0)

    w_copy(0).start()
    x_copy(0, 0).start()
    w_copy(1).start()
    b_copy.start()
    for k in range(2, 2 * num_layers):
        w_copy(k).start()
    for q in range(1, _AHEAD):
        x_copy(0, q).start()

    def body(it, carry):
        def wait_first_iter(copy):
            pl.when(it == 0)(copy.wait)

        for j, n in enumerate(_SIZES):
            if j == 0:
                wait_first_iter(w_copy(0))
                v0 = vbuf[0]
            if j in seg_start:
                q = seg_start.index(j)
                if j != 1:
                    x_copy(it, q).wait()
                if q + _AHEAD < num_segs:
                    x_copy(it, q + _AHEAD).start()
                else:
                    pl.when(it < num_iters - 1)(x_copy(it, q + _AHEAD).start)

            rows = pl.ds(row(it, offs[j]), n)
            if j == 0:
                ha = _mm(xbuf[pl.ds(row(it, 0), _SPLIT), :], v0).astype(jnp.bfloat16)
                ha = hold(ha, 0, _HOLD)
                wait_first_iter(w_copy(1))
                wait_first_iter(b_copy)
                hb = _mm(xbuf[pl.ds(row(it, _SPLIT), n - _SPLIT), :], v0)
                h = jnp.concatenate([ha, hb.astype(jnp.bfloat16)], axis=0)
            x = xbuf[rows, :]
            x0 = x.astype(jnp.float32)

            for l in range(num_layers):
                if j > 0 or l > 0:
                    h = _mm(x, vbuf[l]).astype(jnp.bfloat16)
                if j == 0 and l > 0:
                    h = hold(h, 0, _HOLD)
                    wait_first_iter(w_copy(2 * l + 1))
                g = _mm(h, ubuf[l])
                b = bbuf[pl.ds(l, 1), :].astype(jnp.float32)
                x = (x0 * (g + b) + x.astype(jnp.float32)).astype(jnp.bfloat16)
                if j == 0 and l < num_layers - 1:
                    x = hold(x, 0, _HOLD)
                    wait_first_iter(w_copy(2 * l + 2))

            if j == 0:
                x = hold(x, _HOLD_NEXT, _HOLD)
                x_copy(it, 1).wait()
            if j == num_chunks - 1:
                o = 0
                for p in _LAST_PIECES:
                    obuf[pl.ds(row(it, offs[j] + o), p), :] = x[o : o + p]
                    o_copy(it, offs[j] + o, p).start()
                    o += p
            else:
                obuf[rows, :] = x
                if j in out_first:
                    off = offs[out_first[j]]
                    o_copy(it, off, offs[j + 1] - off).start()
        return carry

    jax.lax.fori_loop(0, num_iters, body, 0)
    pltpu.make_async_copy(o_hbm, o_hbm, osem.at[0]).wait()


@jax.jit
def pallas_standalone__cross_network_dcn_v2__recsys_kernel(x0, U, V, bs):
    B, D = x0.shape
    L, _, R = U.shape
    assert B % sum(_SIZES) == 0, "batch must be a multiple of the unrolled block"
    assert sum(_IN_SEGS) == sum(_OUT_SEGS) == len(_SIZES)
    assert sum(_LAST_PIECES) == _SIZES[-1] and _OUT_SEGS[-1] == 1
    assert _IN_SEGS[:2] == (1, 1) and _AHEAD < len(_IN_SEGS)
    hbm = pl.BlockSpec(memory_space=pl.ANY)
    return pl.pallas_call(
        _cross_kernel,
        in_specs=[hbm] * 4,
        out_specs=hbm,
        out_shape=jax.ShapeDtypeStruct((B, D), x0.dtype),
        scratch_shapes=[
            pltpu.VMEM((B, D), x0.dtype),
            pltpu.VMEM((B, D), x0.dtype),
            pltpu.VMEM((L, D, R), U.dtype),
            pltpu.VMEM((L + 1, R, D), V.dtype),
            pltpu.VMEM((L, D), bs.dtype),
            pltpu.SemaphoreType.DMA((len(_IN_SEGS) + 2 * L + 1,)),
            pltpu.SemaphoreType.DMA((1,)),
        ],
        compiler_params=pltpu.CompilerParams(
            vmem_limit_bytes=100 * 1024 * 1024,
            flags={"XLA_TPU_RESCHEDULE_DMA_DONES": True},
            disable_semaphore_checks=True,
            disable_bounds_checks=True,
        ),
    )(x0, U, V, bs)
```
